```python
import os as _os
_os.environ.setdefault("JAX_PLATFORMS", "cpu")
import jax
import jax.numpy as jnp

def _softmax(x, axis=-1):
    return jax.nn.softmax(x, axis=axis)
def _gelu(x):
    return jax.nn.gelu(x, approximate=True)
def _silu(x):
    return jax.nn.silu(x)
def _sigmoid(x):
    return jax.nn.sigmoid(x)
def _layernorm(x, axis=-1, eps=1e-5):
    m = jnp.mean(x, axis=axis, keepdims=True)
    v = jnp.var(x, axis=axis, keepdims=True)
    return (x - m) / jnp.sqrt(v + eps)
def _scatter_add(tgt, idx, src, axis=0):
    return tgt.at[idx].add(src)
def _segment_sum(src, seg, n):
    return jax.ops.segment_sum(src, seg, n)
class _Rng:
    def __init__(self, key):
        self._k = key
    def _next(self):
        self._k, sub = jax.random.split(self._k)
        return sub
    def normal(self, shape):
        return jax.random.normal(self._next(), shape, dtype=jnp.bfloat16)
    def randint(self, lo, hi, shape):
        return jax.random.randint(self._next(), shape, lo, hi, dtype=jnp.int32)
    def uniform(self, shape, lo=0.0, hi=1.0):
        return jax.random.uniform(self._next(), shape, jnp.bfloat16, lo, hi)
    def permutation(self, n):
        return jax.random.permutation(self._next(), n)


kernel_name = 'standalone__gqa_block_cached__near_ridge'

def setup_inputs():
    _rng = _Rng(jax.random.key(int.from_bytes(__import__("os").urandom(4), "little")))
    _w = (lambda a: (lambda t: t.astype(jnp.bfloat16) if jnp.issubdtype(t.dtype, jnp.floating) else t)(jnp.asarray(a)))
    B, Sq, D = 8, 80, 512
    Hq, Hkv, Sk, Dh = 32, 8, 2048, 128
    assert Hq % Hkv == 0, (Hq, Hkv)
    return {
        "x": _w((lambda *s: _rng.normal(s) * 0.8)(B, Sq, D)),
        "k_cache": _w((lambda *s: _rng.normal(s) * 0.8)(B, Hkv, Sk, Dh)),
        "v_cache": _w((lambda *s: _rng.normal(s) * 0.05)(B, Hkv, Sk, Dh)),
        "wq": _w((lambda *s: _rng.normal(s) * 0.8)(D, Hq * Dh) * (D ** -0.5)),
        "wo": _w((lambda *s: _rng.normal(s) * 0.05)(Hq * Dh, D) * ((Hq * Dh) ** -0.5)),
    }

def reference(x, k_cache, v_cache, wq, wo):
    B, Sq, D = x.shape
    Hq, Dh = 32, 128
    Hkv = k_cache.shape[1]
    rep = Hq // Hkv
    q = (lambda x, *d: x.transpose(*d))((x @ wq).reshape(B, Sq, Hq, Dh), 0, 2, 1, 3)
    k = jnp.repeat(k_cache, rep, axis=1)
    v = jnp.repeat(v_cache, rep, axis=1)
    scores = jnp.einsum("bhqd,bhkd->bhqk", q, k) * (Dh ** -0.5)
    p = _softmax(scores, axis=-1)
    o = jnp.einsum("bhqk,bhkd->bhqd", p, v)
    return (lambda x, *d: x.transpose(*d))(o, 0, 2, 1, 3).reshape(B, Sq, Hq * Dh) @ wo
```

```python
import functools
import jax
import jax.numpy as jnp
from jax import lax
import jax.experimental.pallas as pl
import jax.experimental.pallas.tpu as pltpu

B, SQ, D = 8, 80, 512
HQ, HKV, SK, DH = 32, 8, 2048, 128
REP = HQ // HKV
M = REP * SQ
GW = REP * DH
QSCALE = (DH ** -0.5) * 1.4426950408889634
NT = (((1,), (1,)), ((), ()))
FL = {'rdlp': {'XLA_TPU_RESCHEDULE_DMA_DONES': True, 'XLA_TPU_FORCE_LP_LLO_SCHEDULER': True}, 'rdev': {'XLA_TPU_RESCHEDULE_DMA_DONES': True, 'XLA_TPU_EVENLY_DISTRIBUTE_CRITICAL_NODES': True}, 'lp': {'XLA_TPU_FORCE_LP_LLO_SCHEDULER': True}, 'ev': {'XLA_TPU_EVENLY_DISTRIBUTE_CRITICAL_NODES': True},
      'rd': {'XLA_TPU_RESCHEDULE_DMA_DONES': True}}
BF, F32, U32 = jnp.bfloat16, jnp.float32, jnp.uint32


def build(cw=512, vmem_mb=100, order=1, waits='inline', flags='rdlp', nsb=3, dyn=1, L=2, nodma=0, ng=8, noexp=0, nol=0, nomax=0):
    NC = SK // cw

    def kernel(x_hbm, k_hbm, v_hbm, wq_hbm, wo_hbm, out_hbm,
               x_v, wq_v, wo_v, k_v, v_v, q_v, o_v, acc, out_v, m_v,
               sem, *s_refs):
        class Nop:
            def start(self): pass
            def wait(self): pass

        def k_copy(g, b):
            if nodma: return Nop()
            return pltpu.make_async_copy(k_hbm.at[b, g], k_v.at[g % 2, b], sem.at[(g % 2) * 32 + b])

        def v_copy(g, b):
            if nodma: return Nop()
            return pltpu.make_async_copy(v_hbm.at[b, g], v_v.at[g % 2, b], sem.at[(g % 2) * 32 + 8 + b])

        def wq_copy(g):
            return pltpu.make_async_copy(wq_hbm.at[:, pl.ds(pl.multiple_of(g * GW, GW), GW)], wq_v.at[g % 2], sem.at[(g % 2) * 32 + 16])

        def wo_copy(g):
            return pltpu.make_async_copy(wo_hbm.at[pl.ds(pl.multiple_of(g * GW, GW), GW), :], wo_v.at[g % 2], sem.at[(g % 2) * 32 + 17])

        def ld(ref, sl, b, c):
            w = ref.bitcast(U32)[sl, b, c * cw // 2:(c + 1) * cw // 2, :]
            return pltpu.bitcast(w, BF)

        x_cp = pltpu.make_async_copy(x_hbm, x_v, sem.at[18])
        x_cp.start()
        wq_copy(0).start()
        x_cp.wait()
        k_copy(0, 0).start()
        acc[...] = jnp.zeros_like(acc)

        def group(g, carry):
            sl = g % 2

            def start_kv(copy, bb):
                gg = g + bb // B
                if bb < B:
                    copy(g, bb).start()
                else:
                    @pl.when(gg < ng)
                    def _():
                        copy(gg, bb - B).start()

            wq_copy(g).wait()
            if waits == 'top':
                for b in range(B):
                    k_copy(g, b).wait()
                    v_copy(g, b).wait()
                wo_copy(g).wait()


            @pl.when(g == 0)
            def _():
                for b in range(L):
                    v_copy(0, b).start()
                    k_copy(0, b + 1).start()

            q = jnp.dot(x_v[...], wq_v[sl], preferred_element_type=F32) * QSCALE
            q = q.astype(BF)
            for b in range(B):
                for h in range(REP):
                    qq = q[b * SQ:(b + 1) * SQ, h * DH:(h + 1) * DH]
                    q_v[b, h * SQ // 2:(h + 1) * SQ // 2, :] = pltpu.bitcast(qq, U32)

            def fused(bq, bp):
                st = dict(mx=None, l=None, o=None, p={})
                if bp is not None:
                    start_kv(v_copy, bp + L)
                    start_kv(k_copy, bp + L + 1)
                    if bp == 2:
                        wo_copy(g).start()
                    if bp == 4:
                        @pl.when(g + 1 < ng)
                        def _():
                            wq_copy(g + 1).start()
                if bq is not None:
                    if waits == 'inline':
                        k_copy(g, bq).wait()
                    q = pltpu.bitcast(q_v[bq], BF)
                    s_nxt = s_refs[bq % nsb].at[sl if dyn else 0]
                if bp is not None:
                    if waits == 'inline':
                        v_copy(g, bp).wait()
                    s_cur = s_refs[bp % nsb].at[sl if dyn else 0]
                    m = jnp.max(m_v[sl if dyn else 0, bp % 4], axis=1, keepdims=True)

                def QK(c):
                    if bq is None:
                        R = (B - 1) * SQ
                        w = D // NC
                        o = pltpu.bitcast(o_v[0:R // 2, :], BF)
                        acc[0:R, c * w:(c + 1) * w] += jnp.dot(o, wo_v[sl, :, c * w:(c + 1) * w], preferred_element_type=F32)
                        return
                    s = lax.dot_general(q, ld(k_v, sl, bq, c), NT, preferred_element_type=F32)
                    s_nxt[:, c * cw:(c + 1) * cw] = s
                    for j in range(cw // 128):
                        sj = s[:, j * 128:(j + 1) * 128]
                        st['mx'] = sj if (st['mx'] is None or nomax) else jnp.maximum(st['mx'], sj)
                    if c == NC - 1:
                        m_v[sl if dyn else 0, bq % 4] = st['mx']

                def EX(c):
                    if bp is None or c >= NC: return
                    p = s_cur[:, c * cw:(c + 1) * cw] - m
                    if not noexp: p = jnp.exp2(p)
                    for j in range(cw // 128):
                        pj = p[:, j * 128:(j + 1) * 128]
                        st['l'] = pj if (st['l'] is None or nol) else st['l'] + pj
                    st['p'][c] = p.astype(BF)

                def PV(c):
                    if bp is None: return
                    oc = jnp.dot(st['p'][c], ld(v_v, sl, bp, c), preferred_element_type=F32)
                    st['o'] = oc if st['o'] is None else st['o'] + oc

                def FIN():
                    if bp is None: return
                    l = jnp.sum(st['l'], axis=1, keepdims=True)
                    o = (st['o'] * (1.0 / l)).astype(BF)
                    for h in range(REP):
                        o_v[bp * SQ // 2:(bp + 1) * SQ // 2, h * DH:(h + 1) * DH] = pltpu.bitcast(o[h * SQ:(h + 1) * SQ, :], U32)

                if order == 0:
                    for c in range(NC): QK(c); EX(c); PV(c)
                    FIN()
                elif order == 1:
                    for c in range(NC - 1): QK(c); EX(c); PV(c)
                    EX(NC - 1); PV(NC - 1); FIN(); QK(NC - 1)
                elif order == 2:
                    QK(0); EX(0)
                    for c in range(NC - 1): EX(c + 1); PV(c); QK(c + 1) if c + 1 < NC - 1 else None
                    PV(NC - 1); QK(NC - 1); FIN()

            fused(0, None)
            for b in range(B - 1):
                fused(b + 1, b)
            if waits == 'inline':
                wo_copy(g).wait()
            fused(None, B - 1)
            R = (B - 1) * SQ
            o = pltpu.bitcast(o_v[R // 2:, :], BF)
            acc[R:, :] += jnp.dot(o, wo_v[sl], preferred_element_type=F32)
            return carry

        lax.fori_loop(0, ng, group, 0)
        out_v[...] = acc[...].astype(BF)
        o_cp = pltpu.make_async_copy(out_v, out_hbm, sem.at[19])
        o_cp.start()
        o_cp.wait()

    @jax.jit
    def run(x, k_cache, v_cache, wq, wo):
        any_spec = pl.BlockSpec(memory_space=pl.ANY)
        out = pl.pallas_call(
            kernel,
            out_shape=jax.ShapeDtypeStruct((B * SQ, D), BF),
            in_specs=[any_spec] * 5,
            out_specs=any_spec,
            scratch_shapes=[
                pltpu.VMEM((B * SQ, D), BF),
                pltpu.VMEM((2, D, GW), BF),
                pltpu.VMEM((2, GW, D), BF),
                pltpu.VMEM((2, B, SK, DH), BF),
                pltpu.VMEM((2, B, SK, DH), BF),
                pltpu.VMEM((B, M // 2, DH), U32),
                pltpu.VMEM((B * SQ // 2, GW), U32),
                pltpu.VMEM((B * SQ, D), F32),
                pltpu.VMEM((B * SQ, D), BF),
                pltpu.VMEM((2, 4, M, 128), F32),
                pltpu.SemaphoreType.DMA((64,)),
            ] + [pltpu.VMEM((2, M, SK), F32)] * nsb,
            compiler_params=pltpu.CompilerParams(vmem_limit_bytes=vmem_mb * 1024 * 1024, flags=FL.get(flags)),
        )(x.reshape(B * SQ, D), k_cache, v_cache, wq, wo)
        return out.reshape(B, SQ, D)

    return run


pallas_standalone__gqa_block_cached__near_ridge_kernel = build()
```

```python
import functools
import numpy as np
import jax
import jax.numpy as jnp
from jax import lax
import jax.experimental.pallas as pl
import jax.experimental.pallas.tpu as pltpu

B, SQ, D = 8, 80, 512
HQ, HKV, SK, DH = 32, 8, 2048, 128
REP = HQ // HKV
M = REP * SQ
GW = REP * DH
QSCALE = (DH ** -0.5) * 1.4426950408889634
NT = (((1,), (1,)), ((), ()))
FL = {'rd': {'XLA_TPU_RESCHEDULE_DMA_DONES': True}}
BF, F32, U32 = jnp.bfloat16, jnp.float32, jnp.uint32


def build(cw=512, vmem_mb=100, flags='rd', L=2, rb=16, tie=2, lag=0, fin0=16, finst=4, ng=8, nodma=0, pattern='QQPQPQPP', pace=1, cs=1, nb0=3, kw=2, cwt=3, off=0, fastrcp=1, noqp=0, noop=0, nokv=0):
    NC = SK // cw
    NT_ = SK // 128

    def kernel(x_hbm, k_hbm, v_hbm, wq_hbm, wo_hbm, out_hbm,
               x_v, wq_v, wo_v, k_v, v_v, q_v, o_v, acc, out_v, m_v, l_v, oa_v, zr,
               s0, s1, s2, p0, p1, p2,
               sem):
        ss, pp = (s0, s1, s2), (p0, p1, p2)

        class Nop:
            def start(self): pass
            def wait(self): pass

        def k_copy(g, b):
            if nodma: return Nop()
            return pltpu.make_async_copy(k_hbm.at[b, g], k_v.at[b % 4], sem.at[(g % 2) * 10 + b % 4])

        def v_copy(g, b):
            if nodma: return Nop()
            return pltpu.make_async_copy(v_hbm.at[b, g], v_v.at[b % 4], sem.at[(g % 2) * 10 + 4 + b % 4])

        def wq_copy(g):
            if nodma > 1: return Nop()
            return pltpu.make_async_copy(wq_hbm.at[:, pl.ds(pl.multiple_of(g * GW, GW), GW)], wq_v, sem.at[(g % 2) * 10 + 8])

        def wo_copy(g):
            if nodma > 1: return Nop()
            return pltpu.make_async_copy(wo_hbm.at[pl.ds(pl.multiple_of(g * GW, GW), GW), :], wo_v, sem.at[(g % 2) * 10 + 9])

        def ld(ref, sl, b, c):
            if nokv: b = b % 2
            w = ref.bitcast(U32)[b % 4, c * cw // 2:(c + 1) * cw // 2, :]
            return pltpu.bitcast(w, BF)

        R0 = nb0 * SQ
        R1 = (B - 2) * SQ
        xa_cp = pltpu.make_async_copy(x_hbm.at[pl.ds(0, R0)], x_v.at[pl.ds(0, R0)], sem.at[20])
        xb_cp = pltpu.make_async_copy(x_hbm.at[pl.ds(R0, B * SQ - R0)], x_v.at[pl.ds(R0, B * SQ - R0)], sem.at[21])

        def out_copy(r0, r1, c0, c1, s):
            return pltpu.make_async_copy(out_v.at[pl.ds(r0, r1 - r0), pl.ds(c0, c1 - c0)],
                                         out_hbm.at[pl.ds(r0, r1 - r0), pl.ds(c0, c1 - c0)], sem.at[s])

        out_a, out_b, out_c = out_copy(0, R1, 0, 256, 20), out_copy(0, R1, 256, 512, 21), out_copy(R1, B * SQ, 0, 512, 22)

        wq_copy(0).start()
        xa_cp.start()
        k_copy(0, 0).start()
        xb_cp.start()
        k_copy(0, 1).start()
        v_copy(0, 0).start()
        acc[...] = jnp.zeros_like(acc)
        zr[...] = jnp.zeros_like(zr)
        wq_copy(0).wait()
        xa_cp.wait()

        def group(g, carry):
            sl = g % 2

            def kv_op(copy, bb, what):
                run = lambda cp: cp.start() if what == 'start' else cp.wait()
                if bb < B:
                    run(copy(g, bb))
                else:
                    @pl.when(g + 1 < ng)
                    def _():
                        run(copy(g + 1, bb - B))

            zero = jnp.tile(zr[...], (rb // 8, 1))

            def dep(mv, cv):
                return pltpu.bitcast(pltpu.bitcast(mv, U32) | (pltpu.bitcast(cv, U32) & zero), F32)

            hist = []
            fin_links = {}

            events = []
            NL = (M // rb) * (NT_ // tie)

            def add_events(val):
                for r in range(0, val.shape[0], rb):
                    events.append(val[r:r + rb, 0:128])

            def QP(b0, b1, h):
                q = jnp.dot(x_v[b0 * SQ:b1 * SQ, :], wq_v[:, h * DH:(h + 1) * DH], preferred_element_type=F32) * QSCALE
                if b0 == 0 and h == kw:
                    @pl.when(g == 0)
                    def _():
                        k_copy(0, 0).wait()
                add_events(q)
                q = q.astype(BF)
                for b in range(b0, b1):
                    q_v[sl, b, h * SQ // 2:(h + 1) * SQ // 2, :] = pltpu.bitcast(q[(b - b0) * SQ:(b - b0 + 1) * SQ], U32)

            def QK(b, c):
                q = pltpu.bitcast(q_v[sl, b], BF)
                s = lax.dot_general(q, ld(k_v, sl, b, c), NT, preferred_element_type=F32)
                if c == cs:
                    kv_op(k_copy, b + 2, 'start')
                    kv_op(v_copy, b + 1, 'start')
                    if b == 2:
                        wo_copy(g).start()
                    if b == 3:
                        @pl.when(g + 1 < ng)
                        def _():
                            wq_copy(g + 1).start()
                if c == cwt:
                    kv_op(k_copy, b + 1, 'wait')
                    if b == 0:
                        @pl.when(g == 0)
                        def _():
                            xb_cp.wait()
                    if b >= 1:
                        v_copy(g, b - 1).wait()
                    if b == B - 1:
                        v_copy(g, b).wait()
                        wo_copy(g).wait()

                        @pl.when(g + 1 < ng)
                        def _():
                            wq_copy(g + 1).wait()
                add_events(s)
                ss[b % 3][sl, :, c * cw:(c + 1) * cw] = s
                tt = [s[:, j * 128:(j + 1) * 128] for j in range(cw // 128)]
                while len(tt) > 1: tt = [jnp.maximum(tt[j], tt[j + 1]) for j in range(0, len(tt), 2)]
                if c == 0: m_v[sl, b % 4] = tt[0]
                else: m_v[sl, b % 4] = jnp.maximum(m_v[sl, b % 4], tt[0])

            exs = {}
            pend = {}

            def EXL(b, li, ev):
                ri, jj = divmod(li, NT_ // tie)
                r, j0 = ri * rb, jj * tie
                if jj == 0:
                    exs['m'] = jnp.broadcast_to(jnp.max(m_v[sl, b % 4, r:r + rb, :], axis=1, keepdims=True), (rb, 128))
                    exs['cc'] = None
                deps = list(fin_links.pop((b, li), []))
                if lag and len(hist) >= lag: deps.append(hist[-lag])
                if ev is not None and pace: deps.append(ev)
                mm = exs['m']
                if deps:
                    w = pltpu.bitcast(deps[0], U32)
                    for dd in deps[1:]: w = w | pltpu.bitcast(dd, U32)
                    mm = pltpu.bitcast(pltpu.bitcast(mm, U32) | (w & zero), F32)
                ts = [jnp.exp2(ss[b % 3][sl, r:r + rb, j * 128:(j + 1) * 128] - mm) for j in range(j0, j0 + tie)]
                tt = ts
                while len(tt) > 1: tt = [tt[j] + tt[j + 1] for j in range(0, len(tt), 2)]
                cc = tt[0] if exs['cc'] is None else exs['cc'] + tt[0]
                exs['cc'] = cc
                hist.append(cc)
                pp[b % 3][sl, r:r + rb, j0 * 128:(j0 + tie) * 128] = jnp.concatenate(ts, axis=1).astype(BF)
                if jj == NT_ // tie - 1:
                    l_v[sl, b % 4, r:r + rb, :] = cc

            def PV(b, c):
                oc = jnp.dot(pp[b % 3][sl, :, c * cw:(c + 1) * cw], ld(v_v, sl, b, c), preferred_element_type=F32)
                if (b, c) == (B - 1, 1):
                    @pl.when(g == ng - 1)
                    def _():
                        out_a.start()
                add_events(oc)
                if c == 0: oa_v[sl, b % 2] = oc
                elif c < NC - 1: oa_v[sl, b % 2] += oc
                else:
                    l = jnp.sum(l_v[sl, b % 4], axis=1, keepdims=True)
                    if fastrcp:
                        l = jnp.broadcast_to(l, (M, 128))
                        y = pl.reciprocal(l, approx=True)
                        y = y * (2.0 - l * y)
                    else:
                        y = 1.0 / l
                    o = (oa_v[sl, b % 2] + oc) * y
                    for j in range(M // rb):
                        fin_links.setdefault((b + 2, fin0 + finst * j), []).append(o[j * rb:(j + 1) * rb])
                    o = o.astype(BF)
                    for h in range(REP):
                        o_v[sl, b * SQ:(b + 1) * SQ, h * DH:(h + 1) * DH] = o[h * SQ:(h + 1) * SQ, :]

            def OP(b0, b1, j):
                r = jnp.dot(o_v[sl, b0 * SQ:b1 * SQ, :], wo_v[:, j * 128:(j + 1) * 128], preferred_element_type=F32)
                add_events(r)
                if (b0, j) == (B - 2, 1):
                    @pl.when(g == ng - 1)
                    def _():
                        out_b.start()
                r = acc[b0 * SQ:b1 * SQ, j * 128:(j + 1) * 128] + r
                acc[b0 * SQ:b1 * SQ, j * 128:(j + 1) * 128] = r
                pend[j] = r
                if j % 2 == 1:
                    out_v[b0 * SQ:b1 * SQ, (j - 1) * 128:(j + 1) * 128] = jnp.concatenate(
                        [acc[b0 * SQ:b1 * SQ, (j - 1) * 128:j * 128], r], axis=1).astype(BF)

            P_ = functools.partial
            stages = []
            stages.append(([P_(QP, 0, nb0, h) for h in range(REP)] + [P_(QK, 0, c) for c in range(NC)], None, []))
            stages.append(([P_(QP, nb0, B, h) for h in range(REP)] + [P_(QK, 1, c) for c in range(NC)], 0, [(B - nb0) * SQ] * 4 + [M] * NC))
            for t in range(0, B - 2):
                ops, n = [], dict(P=0, Q=0)
                for ch in pattern:
                    ops.append(P_(PV, t, n['P']) if ch == 'P' else P_(QK, t + 2, n['Q']))
                    n[ch] += 1
                stages.append((ops, t + 1, [M] * (2 * NC)))
            stages.append(([P_(PV, B - 2, 0), P_(OP, 0, B - 2, 0), P_(PV, B - 2, 1), P_(OP, 0, B - 2, 1), P_(PV, B - 2, 2), P_(OP, 0, B - 2, 2), P_(PV, B - 2, 3)],
                  B - 1, [M] * 4 + [(B - 2) * SQ] * 3))
            stages.append(([P_(PV, B - 1, c) for c in range(NC)] + [P_(OP, 0, B - 2, 3)] + [P_(OP, B - 2, B, j) for j in range(4)], None, []))
            flat = [op for st in stages for op in st[0]]
            k = 0
            for ops, exb, sizes in stages:
                total = sum(sizes) // rb
                e0 = len(events)
                li = 0
                for op in ops:
                    op()
                    if exb is None: continue
                    while li < NL and (li * total) // NL - off < len(events) - e0:
                        e = e0 + (li * total) // NL - off
                        EXL(exb, li, events[e] if e >= 0 else None)
                        li += 1
                assert exb is None or li == NL
            return carry

        lax.fori_loop(0, ng, group, 0)
        out_c.start()
        out_a.wait()
        out_b.wait()
        out_c.wait()

    @jax.jit
    def run(x, k_cache, v_cache, wq, wo):
        any_spec = pl.BlockSpec(memory_space=pl.ANY)
        out = pl.pallas_call(
            kernel,
            out_shape=jax.ShapeDtypeStruct((B * SQ, D), BF),
            in_specs=[any_spec] * 5,
            out_specs=any_spec,
            scratch_shapes=[
                pltpu.VMEM((B * SQ, D), BF),
                pltpu.VMEM((D, GW), BF),
                pltpu.VMEM((GW, D), BF),
                pltpu.VMEM((4, SK, DH), BF),
                pltpu.VMEM((4, SK, DH), BF),
                pltpu.VMEM((2, B, M // 2, DH), U32),
                pltpu.VMEM((2, B * SQ, GW), BF),
                pltpu.VMEM((B * SQ, D), F32),
                pltpu.VMEM((B * SQ, D), BF),
                pltpu.VMEM((2, 4, M, 128), F32),
                pltpu.VMEM((2, 4, M, 128), F32),
                pltpu.VMEM((2, 2, M, 128), F32),
                pltpu.VMEM((8, 128), U32),
            ] + [pltpu.VMEM((2, M, SK), F32)] * 3 + [pltpu.VMEM((2, M, SK), BF)] * 3 + [
                pltpu.SemaphoreType.DMA((23,)),
            ],
            compiler_params=pltpu.CompilerParams(vmem_limit_bytes=vmem_mb * 1024 * 1024, flags=FL.get(flags)),
        )(x.reshape(B * SQ, D), k_cache, v_cache, wq, wo)
        return out.reshape(B, SQ, D)

    return run


pallas_standalone__gqa_block_cached__near_ridge_kernel = build()
```

```python
import functools

import jax
from jax import lax
import jax.numpy as jnp
import jax.experimental.pallas as pl
import jax.experimental.pallas.tpu as pltpu

B, SQ, D = 8, 80, 512
HQ, HKV, SK, DH = 32, 8, 2048, 128
REP = HQ // HKV
M = REP * SQ
GW = REP * DH

LANES = 128
CW = 512
NC = SK // CW
RB = 16
TIE = 2
STEPS_PER_ROW_BLOCK = SK // (TIE * LANES)
STEPS = (M // RB) * STEPS_PER_ROW_BLOCK
RING = 4
B_HEAD = 3
B_TAIL = B - 2

QSCALE = (DH ** -0.5) * 1.4426950408889634

BF, F32, U32 = jnp.bfloat16, jnp.float32, jnp.uint32
NT_DIMS = (((1,), (1,)), ((), ()))
SEM_K, SEM_V, SEM_WQ, SEM_WO, NUM_SEMS = 0, RING, 2 * RING, 2 * RING + 1, 2 * RING + 2


def _tree(op, vals):
    while len(vals) > 1:
        vals = [op(vals[i], vals[i + 1]) for i in range(0, len(vals), 2)]
    return vals[0]


def _kernel(x_hbm, k_hbm, v_hbm, wq_hbm, wo_hbm, out_hbm,
            x_v, wq_v, wo_v, k_v, v_v, q_v, o_v, acc, out_v, m_v, l_v, pv_v, zero_v,
            s0, s1, s2, p0, p1, p2, sem):
    s_bufs, p_bufs = (s0, s1, s2), (p0, p1, p2)

    def sem_at(g, i):
        return sem.at[i if isinstance(g, int) else lax.shift_right_logical(g, 3) + i]

    def k_copy(g, b):
        return pltpu.make_async_copy(k_hbm.at[b, g], k_v.at[b % RING], sem_at(g, SEM_K + b % RING))

    def v_copy(g, b):
        return pltpu.make_async_copy(v_hbm.at[b, g], v_v.at[b % RING], sem_at(g, SEM_V + b % RING))

    def wq_copy(g):
        cols = pl.ds(pl.multiple_of(g * GW, GW), GW)
        return pltpu.make_async_copy(wq_hbm.at[:, cols], wq_v, sem_at(g, SEM_WQ))

    def wo_copy(g):
        rows = pl.ds(pl.multiple_of(g * GW, GW), GW)
        return pltpu.make_async_copy(wo_hbm.at[rows, :], wo_v, sem_at(g, SEM_WO))

    def x_copy(r0, r1, s):
        rows = pl.ds(r0, r1 - r0)
        return pltpu.make_async_copy(x_hbm.at[rows], x_v.at[rows], sem.at[s])

    def out_copy(r0, r1, c0, c1, s):
        rows, cols = pl.ds(r0, r1 - r0), pl.ds(c0, c1 - c0)
        return pltpu.make_async_copy(out_v.at[rows, cols], out_hbm.at[rows, cols], sem.at[s])

    x_head = x_copy(0, B_HEAD * SQ, SEM_WO)
    x_rest = x_copy(B_HEAD * SQ, B * SQ, SEM_V + 3)
    out_a = out_copy(0, B_TAIL * SQ, 0, D // 2, SEM_K)
    out_b = out_copy(0, B_TAIL * SQ, D // 2, D, SEM_K + 1)
    out_c = out_copy(B_TAIL * SQ, B * SQ, 0, D, SEM_K + 2)

    wq_copy(0).start()
    x_head.start()
    k_copy(0, 0).start()
    x_rest.start()
    k_copy(0, 1).start()
    v_copy(0, 0).start()
    acc[...] = jnp.zeros_like(acc)
    zero_v[...] = jnp.zeros_like(zero_v)
    wq_copy(0).wait()
    x_head.wait()

    def group(g, carry):
        sl = g % 2
        zero = jnp.tile(zero_v[...], (RB // 8, 1))

        def kv(copy, b, action):
            if b < B:
                action(copy(g, b))
            else:
                @pl.when(g + 1 < HKV)
                def _():
                    action(copy(g + 1, b - B))

        def prefetch(b):
            kv(k_copy, b + 2, lambda c: c.start())
            kv(v_copy, b + 1, lambda c: c.start())
            if b == 2:
                wo_copy(g).start()
            if b == 3:
                @pl.when(g + 1 < HKV)
                def _():
                    wq_copy(g + 1).start()

        def await_inputs(b):
            kv(k_copy, b + 1, lambda c: c.wait())
            if b == 0:
                @pl.when(g == 0)
                def _():
                    x_rest.wait()
            else:
                v_copy(g, b - 1).wait()
            if b == B - 1:
                v_copy(g, b).wait()
                wo_copy(g).wait()

                @pl.when(g + 1 < HKV)
                def _():
                    wq_copy(g + 1).wait()

        events = []
        after = {}
        row = {}

        def record(result):
            for r in range(0, result.shape[0], RB):
                events.append(result[r:r + RB, :LANES])

        def q_proj(b0, b1, h):
            q = jnp.dot(x_v[b0 * SQ:b1 * SQ, :], wq_v[:, h * DH:(h + 1) * DH],
                        preferred_element_type=F32) * QSCALE
            if b0 == 0 and h == 2:
                @pl.when(g == 0)
                def _():
                    k_copy(0, 0).wait()
            record(q)
            q = q.astype(BF)
            for b in range(b0, b1):
                q_v[sl, b, h * SQ // 2:(h + 1) * SQ // 2, :] = pltpu.bitcast(
                    q[(b - b0) * SQ:(b - b0 + 1) * SQ], U32)

        def qk(b, c):
            q = pltpu.bitcast(q_v[sl, b], BF)
            s = lax.dot_general(q, k_v[b % RING, c * CW:(c + 1) * CW, :], NT_DIMS,
                                preferred_element_type=F32)
            if c == 1 and b < 2:
                prefetch(b)
            if c == NC - 1:
                await_inputs(b)
            record(s)
            s_bufs[b % 3][sl, :, c * CW:(c + 1) * CW] = s
            m = _tree(jnp.maximum, [s[:, j:j + LANES] for j in range(0, CW, LANES)])
            m_v[sl, b % 4] = m if c == 0 else jnp.maximum(m_v[sl, b % 4], m)

        def softmax_step(b, step, event):
            rb, jj = divmod(step, STEPS_PER_ROW_BLOCK)
            rows, c0 = slice(rb * RB, (rb + 1) * RB), jj * TIE * LANES
            if jj == 0:
                m = jnp.max(m_v[sl, b % 4, rows, :], axis=1, keepdims=True)
                row["max"], row["sum"] = jnp.broadcast_to(m, (RB, LANES)), None
            pace = functools.reduce(
                jnp.bitwise_or,
                [pltpu.bitcast(v, U32) for v in after.pop((b, step), []) + [event]])
            m = pltpu.bitcast(pltpu.bitcast(row["max"], U32) | (pace & zero), F32)
            p = [jnp.exp2(s_bufs[b % 3][sl, rows, c:c + LANES] - m)
                 for c in range(c0, c0 + TIE * LANES, LANES)]
            total = _tree(jnp.add, p)
            row["sum"] = total if row["sum"] is None else row["sum"] + total
            p_bufs[b % 3][sl, rows, c0:c0 + TIE * LANES] = jnp.concatenate(p, axis=1).astype(BF)
            if jj == STEPS_PER_ROW_BLOCK - 1:
                l_v[sl, b % 4, rows, :] = row["sum"]

        def pv(b, c):
            o = jnp.dot(p_bufs[b % 3][sl, :, c * CW:(c + 1) * CW],
                        v_v[b % RING, c * CW:(c + 1) * CW, :], preferred_element_type=F32)
            if (b, c) == (B - 1, 1):
                @pl.when(g == HKV - 1)
                def _():
                    out_a.start()
            if c == 0 and b + 2 < B:
                prefetch(b + 2)
            record(o)
            if c == 0:
                pv_v[sl, b % 2] = o
            elif c < NC - 1:
                pv_v[sl, b % 2] += o
            else:
                inv_l = 1.0 / jnp.sum(l_v[sl, b % 4], axis=1, keepdims=True)
                o = (pv_v[sl, b % 2] + o) * inv_l
                for j in range(M // RB):
                    after[(b + 2, 16 + 4 * j)] = [o[j * RB:(j + 1) * RB]]
                o = o.astype(BF)
                for h in range(REP):
                    o_v[sl, b * SQ:(b + 1) * SQ, h * DH:(h + 1) * DH] = o[h * SQ:(h + 1) * SQ, :]

        def out_proj(b0, b1, j):
            rows, cols = slice(b0 * SQ, b1 * SQ), slice(j * LANES, (j + 1) * LANES)
            y = jnp.dot(o_v[sl, rows, :], wo_v[:, cols], preferred_element_type=F32)
            record(y)
            if b0 > 0 and j == 1:
                @pl.when(g == HKV - 1)
                def _():
                    out_b.start()
            y = acc[rows, cols] + y
            acc[rows, cols] = y
            if j % 2 == 1:
                left = acc[rows, (j - 1) * LANES:j * LANES]
                out_v[rows, (j - 1) * LANES:(j + 1) * LANES] = jnp.concatenate(
                    [left, y], axis=1).astype(BF)

        def stage(matmuls, unit=None, rows=0):
            first, step = len(events), 0
            for matmul in matmuls:
                matmul()
                while unit is not None and step < STEPS:
                    e = first + (step * (rows // RB)) // STEPS
                    if e >= len(events):
                        break
                    softmax_step(unit, step, events[e])
                    step += 1
            assert unit is None or step == STEPS

        P = functools.partial
        stage([P(q_proj, 0, B_HEAD, h) for h in range(REP)]
              + [P(qk, 0, c) for c in range(NC)])
        stage([P(q_proj, B_HEAD, B, h) for h in range(REP)]
              + [P(qk, 1, c) for c in range(NC)],
              unit=0, rows=REP * (B - B_HEAD) * SQ + NC * M)
        for t in range(B - 2):
            stage([P(qk, t + 2, 0), P(qk, t + 2, 1), P(pv, t, 0), P(qk, t + 2, 2),
                   P(pv, t, 1), P(qk, t + 2, 3), P(pv, t, 2), P(pv, t, 3)],
                  unit=t + 1, rows=2 * NC * M)
        stage([P(pv, B - 2, 0), P(out_proj, 0, B_TAIL, 0), P(pv, B - 2, 1),
               P(out_proj, 0, B_TAIL, 1), P(pv, B - 2, 2), P(out_proj, 0, B_TAIL, 2),
               P(pv, B - 2, 3)],
              unit=B - 1, rows=NC * M + 3 * B_TAIL * SQ)
        stage([P(pv, B - 1, c) for c in range(NC)] + [P(out_proj, 0, B_TAIL, 3)]
              + [P(out_proj, B_TAIL, B, j) for j in range(D // LANES)])
        return carry

    lax.fori_loop(0, HKV, group, 0)
    out_c.start()
    out_a.wait()
    out_b.wait()
    out_c.wait()


@jax.jit
def pallas_standalone__gqa_block_cached__near_ridge_kernel(
    x: jax.Array,
    k_cache: jax.Array,
    v_cache: jax.Array,
    wq: jax.Array,
    wo: jax.Array,
):
    assert x.shape == (B, SQ, D) and k_cache.shape == v_cache.shape == (B, HKV, SK, DH)
    assert wq.shape == (D, HQ * DH) and wo.shape == (HQ * DH, D)
    hbm = pl.BlockSpec(memory_space=pl.ANY)
    out = pl.pallas_call(
        _kernel,
        out_shape=jax.ShapeDtypeStruct((B * SQ, D), BF),
        in_specs=[hbm] * 5,
        out_specs=hbm,
        scratch_shapes=[
            pltpu.VMEM((B * SQ, D), BF),
            pltpu.VMEM((D, GW), BF),
            pltpu.VMEM((GW, D), BF),
            pltpu.VMEM((RING, SK, DH), BF),
            pltpu.VMEM((RING, SK, DH), BF),
            pltpu.VMEM((2, B, M // 2, DH), U32),
            pltpu.VMEM((2, B * SQ, GW), BF),
            pltpu.VMEM((B * SQ, D), F32),
            pltpu.VMEM((B * SQ, D), BF),
            pltpu.VMEM((2, 4, M, LANES), F32),
            pltpu.VMEM((2, 4, M, LANES), F32),
            pltpu.VMEM((2, 2, M, LANES), F32),
            pltpu.VMEM((8, LANES), U32),
        ]
        + [pltpu.VMEM((2, M, SK), F32)] * 3
        + [pltpu.VMEM((2, M, SK), BF)] * 3
        + [pltpu.SemaphoreType.DMA((NUM_SEMS,))],
        compiler_params=pltpu.CompilerParams(
            vmem_limit_bytes=100 * 1024 * 1024,
            flags={"XLA_TPU_RESCHEDULE_DMA_DONES": True},
        ),
    )(x.reshape(B * SQ, D), k_cache, v_cache, wq, wo)
    return out.reshape(B, SQ, D)
```
